```python
import os as _os
_os.environ.setdefault("JAX_PLATFORMS", "cpu")
import jax
import jax.numpy as jnp

def _softmax(x, axis=-1):
    return jax.nn.softmax(x, axis=axis)
def _gelu(x):
    return jax.nn.gelu(x, approximate=True)
def _silu(x):
    return jax.nn.silu(x)
def _sigmoid(x):
    return jax.nn.sigmoid(x)
def _layernorm(x, axis=-1, eps=1e-5):
    m = jnp.mean(x, axis=axis, keepdims=True)
    v = jnp.var(x, axis=axis, keepdims=True)
    return (x - m) / jnp.sqrt(v + eps)
def _scatter_add(tgt, idx, src, axis=0):
    return tgt.at[idx].add(src)
def _segment_sum(src, seg, n):
    return jax.ops.segment_sum(src, seg, n)
class _Rng:
    def __init__(self, key):
        self._k = key
    def _next(self):
        self._k, sub = jax.random.split(self._k)
        return sub
    def normal(self, shape):
        return jax.random.normal(self._next(), shape, dtype=jnp.bfloat16)
    def randint(self, lo, hi, shape):
        return jax.random.randint(self._next(), shape, lo, hi, dtype=jnp.int32)
    def uniform(self, shape, lo=0.0, hi=1.0):
        return jax.random.uniform(self._next(), shape, jnp.bfloat16, lo, hi)
    def permutation(self, n):
        return jax.random.permutation(self._next(), n)


kernel_name = 'standalone__gqa_softmax__near_ridge'

def setup_inputs():
    _rng = _Rng(jax.random.key(int.from_bytes(__import__("os").urandom(4), "little")))
    _w = (lambda a: (lambda t: t.astype(jnp.bfloat16) if jnp.issubdtype(t.dtype, jnp.floating) else t)(jnp.asarray(a)))
    B, Hq, Hkv, Sq, Sk, D = 8, 16, 8, 512, 512, 256
    return {
        "q": _w((lambda *s: _rng.normal(s) * 0.4)(B, Hq, Sq, D)),
        "k": _w((lambda *s: _rng.normal(s) * 0.4)(B, Hkv, Sk, D)),
        "v": _w((lambda *s: _rng.normal(s) * 0.05)(B, Hkv, Sk, D)),
    }

def reference(q, k, v):
    B, Hq, Sq, D = q.shape
    Hkv = k.shape[1]
    rep = Hq // Hkv
    k = jnp.repeat(k, rep, axis=1)
    v = jnp.repeat(v, rep, axis=1)
    scale = D ** -0.5
    scores = jnp.einsum("bhqd,bhkd->bhqk", q, k) * scale
    p = _softmax(scores, axis=-1)
    return jnp.einsum("bhqk,bhkd->bhqd", p, v)
```

```python
import math

import jax
import jax.numpy as jnp
import jax.experimental.pallas as pl
import jax.experimental.pallas.tpu as pltpu

LANES = 128
CHUNK = 128
LAG = 2
GROUPS_PER_STEP = 8
RAMP = (1, 1, 2, 4)
FIRST_ROWS = 512
N_IN_SEMS = 3
KEY_PARTS = 2


def _pipeline_ops(n_items):
    ops = []
    for i in range(n_items):
        ops += [("qk", i), ("sm", i)]
        if i >= LAG:
            ops.append(("pv", i - LAG))
    ops += [("pv", i) for i in range(max(0, n_items - LAG), n_items)]
    return ops


def _ramp_ops(items_per_group):
    starts = [FIRST_ROWS // CHUNK]
    acc = 0
    for r in RAMP[:-1]:
        acc += r
        starts.append(acc * items_per_group)
    out = [("wait", 0)]
    early_pv = []
    hoisted = None
    nxt = 0
    for kind, i in _pipeline_ops(sum(RAMP) * items_per_group):
        if kind == "qk" and nxt < len(starts) and i == starts[nxt]:
            out.remove(("sm", i - 1))
            out += [("wait", nxt + 1), ("sm", i - 1)]
            if nxt == 0:
                out += early_pv
            else:
                hoisted = i - LAG
                out.append(("pv", hoisted))
            nxt += 1
        if kind == "pv" and nxt == 0:
            early_pv.append((kind, i))
        elif kind == "pv" and i == hoisted:
            pass
        else:
            out.append((kind, i))
    return out


@jax.jit
def pallas_standalone__gqa_softmax__near_ridge_kernel(
    q: jax.Array,
    k: jax.Array,
    v: jax.Array,
):
    B, Hq, Sq, D = q.shape
    Hkv, Sk = k.shape[1], k.shape[2]
    rep = Hq // Hkv
    n_groups = B * Hkv
    tq = rep * Sq
    G = GROUPS_PER_STEP
    R = sum(RAMP)
    n_steps = (n_groups - R) // G
    n_half = D // LANES
    nc = tq // CHUNK
    slots = R + 2 * G
    assert R + n_steps * G == n_groups and n_steps >= 2 and RAMP[0] == 1
    assert D % LANES == 0 and tq % CHUNK == 0 and Sk % (KEY_PARTS * LANES) == 0
    assert FIRST_ROWS % CHUNK == 0 and LAG * CHUNK <= FIRST_ROWS < tq
    exp2_scale = (D ** -0.5) * math.log2(math.e)

    def kernel(q_hbm, k_hbm, v_hbm, o_hbm, q_buf, k_buf, v_buf, o_buf, in_sems, out_sems):
        def fetch(hbm, buf, n0, slot0, cnt, sem, r0=0, nr=None):
            nr = hbm.shape[1] if nr is None else nr
            return [
                pltpu.make_async_copy(
                    hbm.at[pl.ds(n0, cnt), pl.ds(r0, nr), pl.ds(h * LANES, LANES)],
                    buf.at[h, pl.ds(slot0, cnt), pl.ds(r0, nr)],
                    sem,
                )
                for h in range(n_half)
            ]

        def fetch_groups(n0, slot0, cnt, sem):
            return (fetch(k_hbm, k_buf, n0, slot0, cnt, sem)
                    + fetch(q_hbm, q_buf, n0, slot0, cnt, sem)
                    + fetch(v_hbm, v_buf, n0, slot0, cnt, sem))

        def qk(slot, c):
            rows = pl.ds(c * CHUNK, CHUNK)
            qs = [q_buf[h, slot, rows, :] for h in range(n_half)]
            nk = Sk // KEY_PARTS
            parts = []
            for j in range(KEY_PARTS):
                acc = None
                for h in range(n_half):
                    d = jax.lax.dot_general(
                        qs[h], k_buf[h, slot, pl.ds(j * nk, nk), :],
                        (((1,), (1,)), ((), ())), preferred_element_type=jnp.float32)
                    acc = d if acc is None else acc + d
                parts.append(acc)
            return jnp.concatenate(parts, axis=1)

        def softmax(s):
            m = jnp.max(s, axis=-1, keepdims=True)
            p = jnp.exp2((s - m) * exp2_scale)
            l = jnp.sum(p, axis=-1, keepdims=True)
            r = pl.reciprocal(l, approx=True)
            r = r * (2.0 - l * r)
            return (p * r).astype(v_buf.dtype)

        def pv(slot, c, p, n, osem):
            rows = pl.ds(c * CHUNK, CHUNK)
            for h in range(n_half):
                o = jnp.dot(p, v_buf[h, slot], preferred_element_type=jnp.float32)
                o_buf[h, slot, rows, :] = o.astype(o_buf.dtype)
                if osem is not None:
                    pltpu.make_async_copy(
                        o_buf.at[h, slot, rows],
                        o_hbm.at[n, rows, pl.ds(h * LANES, LANES)],
                        osem,
                    ).start()

        def run(ops, n0, slot0, osem, hooks):
            vals = {}
            for kind, i in ops:
                if kind == "wait":
                    hooks["wait"](i)
                    continue
                g, c = divmod(i, nc)
                if kind == "qk":
                    vals[i] = qk(slot0 + g, c)
                    if (kind, i) in hooks:
                        hooks[(kind, i)]()
                elif kind == "sm":
                    vals[i] = softmax(vals[i])
                else:
                    pv(slot0 + g, c, vals.pop(i), n0 + g, osem)

        def wait_out(half):
            r = o_buf.at[:, pl.ds(R + half * G, G)]
            pltpu.make_async_copy(r, r, out_sems.at[half]).wait()

        last_half = (n_steps - 1) % 2
        ramp_out = [
            pltpu.make_async_copy(
                o_buf.at[h, pl.ds(0, R)],
                o_hbm.at[pl.ds(0, R), :, pl.ds(h * LANES, LANES)],
                out_sems.at[last_half],
            )
            for h in range(n_half)
        ]

        makers = [
            lambda s: (fetch(k_hbm, k_buf, 0, 0, 1, s)
                       + fetch(q_hbm, q_buf, 0, 0, 1, s, 0, FIRST_ROWS)),
            lambda s: (fetch(v_hbm, v_buf, 0, 0, 1, s)
                       + fetch(q_hbm, q_buf, 0, 0, 1, s, FIRST_ROWS, tq - FIRST_ROWS)),
        ]
        acc = 1
        for r in RAMP[1:]:
            makers.append(lambda s, a=acc, r=r: fetch_groups(a, a, r, s))
            acc += r
        makers.append(lambda s: fetch_groups(R, R, G, s))
        n_batches = len(makers)

        def batch(b):
            return makers[b](in_sems.at[b % N_IN_SEMS])

        step_sem = in_sems.at[(n_batches - 1) % N_IN_SEMS]

        def ramp_wait(b):
            for c in batch(b):
                c.wait()
            if b + N_IN_SEMS < n_batches:
                for c in batch(b + N_IN_SEMS):
                    c.start()

        def step(t, carry):
            @pl.when(t == 0)
            def _():
                for b in range(N_IN_SEMS):
                    for c in batch(b):
                        c.start()
                run(_ramp_ops(nc), 0, 0, None, {"wait": ramp_wait})

            half = jnp.bitwise_and(t, 1)
            slot0 = R + half * G
            for c in fetch_groups(0, slot0, G, step_sem):
                c.wait()

            @pl.when(t >= 2)
            def _():
                wait_out(half)

            def prefetch():
                @pl.when(t + 1 < n_steps)
                def _():
                    for c in fetch_groups(R + (t + 1) * G, R + (1 - half) * G, G, step_sem):
                        c.start()

                @pl.when(t + 1 == n_steps)
                def _():
                    for c in ramp_out:
                        c.start()

            run(_pipeline_ops(G * nc), R + t * G, slot0, out_sems.at[half],
                {("qk", 1): prefetch})
            return carry

        jax.lax.fori_loop(0, n_steps, step, 0)
        wait_out(1 - last_half)
        for c in ramp_out:
            c.wait()
        wait_out(last_half)

    out = pl.pallas_call(
        kernel,
        in_specs=[pl.BlockSpec(memory_space=pl.ANY)] * 3,
        out_specs=pl.BlockSpec(memory_space=pl.ANY),
        out_shape=jax.ShapeDtypeStruct((n_groups, tq, D), q.dtype),
        scratch_shapes=[
            pltpu.VMEM((n_half, slots, tq, LANES), q.dtype),
            pltpu.VMEM((n_half, slots, Sk, LANES), k.dtype),
            pltpu.VMEM((n_half, slots, Sk, LANES), v.dtype),
            pltpu.VMEM((n_half, slots, tq, LANES), q.dtype),
            pltpu.SemaphoreType.DMA((N_IN_SEMS,)),
            pltpu.SemaphoreType.DMA((2,)),
        ],
        compiler_params=pltpu.CompilerParams(
            vmem_limit_bytes=64 * 1024 * 1024,
            disable_bounds_checks=True,
        ),
    )(
        q.reshape(n_groups, tq, D),
        k.reshape(n_groups, Sk, D),
        v.reshape(n_groups, Sk, D),
    )
    return out.reshape(B, Hq, Sq, D)
```

```python
import math

import jax
import jax.numpy as jnp
import jax.experimental.pallas as pl
import jax.experimental.pallas.tpu as pltpu

LANES = 128
CHUNK = 128
LAG = 2
GROUPS_PER_STEP = 8
RAMP = (1, 1, 2, 4)
FIRST_ROWS = 512
N_IN_SEMS = 3
KEY_PARTS = 2


def _pipeline_ops(n_items):
    ops = []
    for i in range(n_items):
        ops += [("qk", i), ("sm", i)]
        if i >= LAG:
            ops.append(("pv", i - LAG))
    ops += [("pv", i) for i in range(max(0, n_items - LAG), n_items)]
    return ops


def _step_ops(n_items):
    ops = [op for op in _pipeline_ops(n_items) if op[1] != 2]
    ops[ops.index(("qk", 1))] = ("qk2", 1)
    return ops


def _ramp_ops(items_per_group):
    starts = [FIRST_ROWS // CHUNK]
    acc = 0
    for r in RAMP[:-1]:
        acc += r
        starts.append(acc * items_per_group)
    out = [("wait", 0)]
    early_pv = []
    hoisted = None
    nxt = 0
    for kind, i in _pipeline_ops(sum(RAMP) * items_per_group):
        if kind == "qk" and nxt < len(starts) and i == starts[nxt]:
            out.remove(("sm", i - 1))
            out += [("wait", nxt + 1), ("sm", i - 1)]
            if nxt == 0:
                out += early_pv
            else:
                hoisted = i - LAG
                out.append(("pv", hoisted))
            nxt += 1
        if kind == "pv" and nxt == 0:
            early_pv.append((kind, i))
        elif kind == "pv" and i == hoisted:
            pass
        else:
            out.append((kind, i))
    return out


@jax.jit
def pallas_standalone__gqa_softmax__near_ridge_kernel(
    q: jax.Array,
    k: jax.Array,
    v: jax.Array,
):
    B, Hq, Sq, D = q.shape
    Hkv, Sk = k.shape[1], k.shape[2]
    rep = Hq // Hkv
    n_groups = B * Hkv
    tq = rep * Sq
    G = GROUPS_PER_STEP
    R = sum(RAMP)
    n_steps = (n_groups - R) // G
    n_half = D // LANES
    nc = tq // CHUNK
    slots = R + 2 * G
    assert R + n_steps * G == n_groups and n_steps >= 2 and RAMP[0] == 1
    assert D % LANES == 0 and tq % CHUNK == 0 and Sk % (KEY_PARTS * LANES) == 0
    assert FIRST_ROWS % CHUNK == 0 and LAG * CHUNK <= FIRST_ROWS < tq
    assert LAG == 2 and nc >= 3
    exp2_scale = (D ** -0.5) * math.log2(math.e)

    def kernel(q_hbm, k_hbm, v_hbm, o_hbm, q_buf, k_buf, v_buf, o_buf, in_sems, out_sems):
        def fetch(hbm, buf, n0, slot0, cnt, sem, r0=0, nr=None):
            nr = hbm.shape[1] if nr is None else nr
            return [
                pltpu.make_async_copy(
                    hbm.at[pl.ds(n0, cnt), pl.ds(r0, nr), pl.ds(h * LANES, LANES)],
                    buf.at[h, pl.ds(slot0, cnt), pl.ds(r0, nr)],
                    sem,
                )
                for h in range(n_half)
            ]

        def fetch_groups(n0, slot0, cnt, sem):
            return (fetch(k_hbm, k_buf, n0, slot0, cnt, sem)
                    + fetch(q_hbm, q_buf, n0, slot0, cnt, sem)
                    + fetch(v_hbm, v_buf, n0, slot0, cnt, sem))

        def qk(slot, c, n_chunks):
            rows = pl.ds(c * CHUNK, n_chunks * CHUNK)
            qs = [q_buf[h, slot, rows, :] for h in range(n_half)]
            nk = Sk // KEY_PARTS
            parts = []
            for j in reversed(range(KEY_PARTS)):
                acc = None
                for h in range(n_half):
                    d = jax.lax.dot_general(
                        qs[h], k_buf[h, slot, pl.ds(j * nk, nk), :],
                        (((1,), (1,)), ((), ())), preferred_element_type=jnp.float32)
                    acc = d if acc is None else acc + d
                parts.append(acc)
            return jnp.concatenate(parts[::-1], axis=1)

        def softmax(s):
            m = jnp.max(s, axis=-1, keepdims=True)
            p = jnp.exp2((s - m) * exp2_scale)
            l = jnp.sum(p, axis=-1, keepdims=True)
            r = pl.reciprocal(l, approx=True)
            r = r * (2.0 - l * r)
            return (p * r).astype(v_buf.dtype)

        def pv(slot, c, p, n, osem):
            rows = pl.ds(c * CHUNK, p.shape[0])
            for h in range(n_half):
                o = jnp.dot(p, v_buf[h, slot], preferred_element_type=jnp.float32)
                o_buf[h, slot, rows, :] = o.astype(o_buf.dtype)
                if osem is not None:
                    pltpu.make_async_copy(
                        o_buf.at[h, slot, rows],
                        o_hbm.at[n, rows, pl.ds(h * LANES, LANES)],
                        osem,
                    ).start()

        def run(ops, n0, slot0, osem, hooks):
            vals = {}
            for kind, i in ops:
                if kind == "wait":
                    hooks["wait"](i)
                    continue
                g, c = divmod(i, nc)
                if kind in ("qk", "qk2"):
                    vals[i] = qk(slot0 + g, c, 2 if kind == "qk2" else 1)
                    if (kind, i) in hooks:
                        hooks[(kind, i)]()
                elif kind == "sm":
                    vals[i] = softmax(vals[i])
                else:
                    pv(slot0 + g, c, vals.pop(i), n0 + g, osem)

        def wait_out(half):
            r = o_buf.at[:, pl.ds(R + half * G, G)]
            pltpu.make_async_copy(r, r, out_sems.at[half]).wait()

        last_half = (n_steps - 1) % 2
        ramp_out = [
            pltpu.make_async_copy(
                o_buf.at[h, pl.ds(0, R)],
                o_hbm.at[pl.ds(0, R), :, pl.ds(h * LANES, LANES)],
                out_sems.at[last_half],
            )
            for h in range(n_half)
        ]

        makers = [
            lambda s: (fetch(k_hbm, k_buf, 0, 0, 1, s)
                       + fetch(q_hbm, q_buf, 0, 0, 1, s, 0, FIRST_ROWS)),
            lambda s: (fetch(v_hbm, v_buf, 0, 0, 1, s)
                       + fetch(q_hbm, q_buf, 0, 0, 1, s, FIRST_ROWS, tq - FIRST_ROWS)),
        ]
        acc = 1
        for r in RAMP[1:]:
            makers.append(lambda s, a=acc, r=r: fetch_groups(a, a, r, s))
            acc += r
        makers.append(lambda s: fetch_groups(R, R, G, s))
        n_batches = len(makers)

        def batch(b):
            return makers[b](in_sems.at[b % N_IN_SEMS])

        step_sem = in_sems.at[(n_batches - 1) % N_IN_SEMS]

        def ramp_wait(b):
            for c in batch(b):
                c.wait()
            if b + N_IN_SEMS < n_batches:
                for c in batch(b + N_IN_SEMS):
                    c.start()

        def step(t, carry):
            @pl.when(t == 0)
            def _():
                for b in range(N_IN_SEMS):
                    for c in batch(b):
                        c.start()
                run(_ramp_ops(nc), 0, 0, None, {"wait": ramp_wait})

            half = jnp.bitwise_and(t, 1)
            slot0 = R + half * G
            for c in fetch_groups(R + t * G, slot0, G, step_sem):
                c.wait()

            @pl.when(t >= 2)
            def _():
                wait_out(half)

            def prefetch():
                @pl.when(t + 1 < n_steps)
                def _():
                    for c in fetch_groups(R + (t + 1) * G, R + (1 - half) * G, G, step_sem):
                        c.start()

                @pl.when(t + 1 == n_steps)
                def _():
                    for c in ramp_out:
                        c.start()

            run(_step_ops(G * nc), R + t * G, slot0, out_sems.at[half],
                {("qk", 0): prefetch})
            return carry

        jax.lax.fori_loop(0, n_steps, step, 0)
        wait_out(1 - last_half)
        for c in ramp_out:
            c.wait()
        wait_out(last_half)

    out = pl.pallas_call(
        kernel,
        in_specs=[pl.BlockSpec(memory_space=pl.ANY)] * 3,
        out_specs=pl.BlockSpec(memory_space=pl.ANY),
        out_shape=jax.ShapeDtypeStruct((n_groups, tq, D), q.dtype),
        scratch_shapes=[
            pltpu.VMEM((n_half, slots, tq, LANES), q.dtype),
            pltpu.VMEM((n_half, slots, Sk, LANES), k.dtype),
            pltpu.VMEM((n_half, slots, Sk, LANES), v.dtype),
            pltpu.VMEM((n_half, slots, tq, LANES), q.dtype),
            pltpu.SemaphoreType.DMA((N_IN_SEMS,)),
            pltpu.SemaphoreType.DMA((2,)),
        ],
        compiler_params=pltpu.CompilerParams(
            vmem_limit_bytes=64 * 1024 * 1024,
            disable_bounds_checks=True,
        ),
    )(
        q.reshape(n_groups, tq, D),
        k.reshape(n_groups, Sk, D),
        v.reshape(n_groups, Sk, D),
    )
    return out.reshape(B, Hq, Sq, D)
```
